```python
import os as _os
_os.environ.setdefault("JAX_PLATFORMS", "cpu")
import jax
import jax.numpy as jnp

def _softmax(x, axis=-1):
    return jax.nn.softmax(x, axis=axis)
def _gelu(x):
    return jax.nn.gelu(x, approximate=True)
def _silu(x):
    return jax.nn.silu(x)
def _sigmoid(x):
    return jax.nn.sigmoid(x)
def _layernorm(x, axis=-1, eps=1e-5):
    m = jnp.mean(x, axis=axis, keepdims=True)
    v = jnp.var(x, axis=axis, keepdims=True)
    return (x - m) / jnp.sqrt(v + eps)
def _scatter_add(tgt, idx, src, axis=0):
    return tgt.at[idx].add(src)
def _segment_sum(src, seg, n):
    return jax.ops.segment_sum(src, seg, n)
class _Rng:
    def __init__(self, key):
        self._k = key
    def _next(self):
        self._k, sub = jax.random.split(self._k)
        return sub
    def normal(self, shape):
        return jax.random.normal(self._next(), shape, dtype=jnp.bfloat16)
    def randint(self, lo, hi, shape):
        return jax.random.randint(self._next(), shape, lo, hi, dtype=jnp.int32)
    def uniform(self, shape, lo=0.0, hi=1.0):
        return jax.random.uniform(self._next(), shape, jnp.bfloat16, lo, hi)
    def permutation(self, n):
        return jax.random.permutation(self._next(), n)


kernel_name = 'concat_heads__sliding_block_cached__sliding_block_cached__decode'

def setup_inputs():
    _rng = _Rng(jax.random.key(int.from_bytes(__import__("os").urandom(4), "little")))
    _w = (lambda a: (lambda t: t.astype(jnp.bfloat16) if jnp.issubdtype(t.dtype, jnp.floating) else t)(jnp.asarray(a)))
    def _A_setup():
        B, Sq, D = 4, 1, 576
        Hq, Hkv, Sk, Dh = 32, 16, 8192, 128
        assert Hq % Hkv == 0, (Hq, Hkv)
        return {
            "x": _w((lambda *s: _rng.normal(s) * 0.8)(B, Sq, D)),
            "k_cache": _w((lambda *s: _rng.normal(s) * 0.8)(B, Hkv, Sk, Dh)),
            "v_cache": _w((lambda *s: _rng.normal(s) * 0.05)(B, Hkv, Sk, Dh)),
            "wq": _w((lambda *s: _rng.normal(s) * 0.8)(D, Hq * Dh) * (D ** -0.5)),
            "wo": _w((lambda *s: _rng.normal(s) * 0.05)(Hq * Dh, D) * ((Hq * Dh) ** -0.5)),
        }
    _A_in = _A_setup()

    def _B_setup():
        B, Sq, D = 4, 1, 576
        Hq, Hkv, Sk, Dh = 32, 16, 8192, 128
        assert Hq % Hkv == 0, (Hq, Hkv)
        return {
            "x": _w((lambda *s: _rng.normal(s) * 0.8)(B, Sq, D)),
            "k_cache": _w((lambda *s: _rng.normal(s) * 0.8)(B, Hkv, Sk, Dh)),
            "v_cache": _w((lambda *s: _rng.normal(s) * 0.05)(B, Hkv, Sk, Dh)),
            "wq": _w((lambda *s: _rng.normal(s) * 0.8)(D, Hq * Dh) * (D ** -0.5)),
            "wo": _w((lambda *s: _rng.normal(s) * 0.05)(Hq * Dh, D) * ((Hq * Dh) ** -0.5)),
        }
    _B_in = _B_setup()

    return {
        "A_x": _A_in["x"],
        "A_k_cache": _A_in["k_cache"],
        "A_v_cache": _A_in["v_cache"],
        "A_wq": _A_in["wq"],
        "A_wo": _A_in["wo"],
        "B_x": _B_in["x"],
        "B_k_cache": _B_in["k_cache"],
        "B_v_cache": _B_in["v_cache"],
        "B_wq": _B_in["wq"],
        "B_wo": _B_in["wo"],
    }

def reference(A_x, A_k_cache, A_v_cache, A_wq, A_wo, B_x, B_k_cache, B_v_cache, B_wq, B_wo):
    def _A_ref(x, k_cache, v_cache, wq, wo):
        B, Sq, D = x.shape
        Hq, Dh = 32, 128
        Hkv, Sk = k_cache.shape[1], k_cache.shape[2]
        W = min(4096, max(256, Sk // 4))
        rep = Hq // Hkv
        q = (lambda x, *d: x.transpose(*d))((x @ wq).reshape(B, Sq, Hq, Dh), 0, 2, 1, 3)
        k = jnp.repeat(k_cache[:, :, Sk - W:, :], rep, axis=1)
        v = jnp.repeat(v_cache[:, :, Sk - W:, :], rep, axis=1)
        scores = jnp.einsum("bhqd,bhkd->bhqk", q, k) * (Dh ** -0.5)
        p = _softmax(scores, axis=-1)
        o = jnp.einsum("bhqk,bhkd->bhqd", p, v)
        return (lambda x, *d: x.transpose(*d))(o, 0, 2, 1, 3).reshape(B, Sq, Hq * Dh) @ wo

    def _B_ref(x, k_cache, v_cache, wq, wo):
        B, Sq, D = x.shape
        Hq, Dh = 32, 128
        Hkv, Sk = k_cache.shape[1], k_cache.shape[2]
        W = min(4096, max(256, Sk // 4))
        rep = Hq // Hkv
        q = (lambda x, *d: x.transpose(*d))((x @ wq).reshape(B, Sq, Hq, Dh), 0, 2, 1, 3)
        k = jnp.repeat(k_cache[:, :, Sk - W:, :], rep, axis=1)
        v = jnp.repeat(v_cache[:, :, Sk - W:, :], rep, axis=1)
        scores = jnp.einsum("bhqd,bhkd->bhqk", q, k) * (Dh ** -0.5)
        p = _softmax(scores, axis=-1)
        o = jnp.einsum("bhqk,bhkd->bhqd", p, v)
        return (lambda x, *d: x.transpose(*d))(o, 0, 2, 1, 3).reshape(B, Sq, Hq * Dh) @ wo

    a = _A_ref(A_x, A_k_cache, A_v_cache, A_wq, A_wo)
    b = _B_ref(B_x, B_k_cache, B_v_cache, B_wq, B_wo)
    return jnp.concatenate([a, b], axis=-1)
```

```python
import jax
import jax.numpy as jnp
from jax import lax
import jax.experimental.pallas as pl
import jax.experimental.pallas.tpu as pltpu

_HQ, _DH = 32, 128
_PIECE = 128
_CHUNK = 256
_NT = (((1,), (1,)), ((), ()))
_NN = (((1,), (0,)), ((), ()))


@jax.jit
def pallas_concat_heads__sliding_block_cached__sliding_block_cached__decode_kernel(
    A_x: jax.Array,
    A_k_cache: jax.Array,
    A_v_cache: jax.Array,
    A_wq: jax.Array,
    A_wo: jax.Array,
    B_x: jax.Array,
    B_k_cache: jax.Array,
    B_v_cache: jax.Array,
    B_wq: jax.Array,
    B_wo: jax.Array,
):
    nb, sq, d = A_x.shape
    _, hkv, sk, dh = A_k_cache.shape
    win = min(4096, max(256, sk // 4))
    lo = sk - win
    rep = _HQ // hkv
    hw = rep * dh
    rows = rep * nb
    assert (sq, dh, rep, rows) == (1, _DH, 2, 8)
    assert win % (2 * _PIECE) == 0 and win % _CHUNK == 0 and d % (16 * nb) == 0
    wrows = d // nb
    wsplit = wrows // 32 * 16
    nchunk = win // _CHUNK
    f32, dt = jnp.float32, A_x.dtype

    def kernel(xa, ka, va, wqa, woa, xb, kb, vb, wqb, wob, o_ref,
               kv, wbuf, xbuf, sbuf, pbuf, acc, kvsem, wsem, xsem):
        caches = (ka, va, kb, vb)
        weights = (woa, wqb, wob, wqa)
        row = lax.broadcasted_iota(jnp.int32, (rows, dh), 0)

        def weight_pair(m, h, b):
            def start(r, n, priority):
                r0 = pl.multiple_of(b * wrows + r, 16)
                pltpu.make_async_copy(
                    weights[m].at[pl.ds(r0, n), pl.ds(pl.multiple_of(h * hw, hw), hw)],
                    wbuf.at[m, h, pl.ds(r0, n), :],
                    wsem.at[m],
                ).start(priority=priority)

            start(0, wsplit, 0)
            start(wsplit, wrows - wsplit, 1)

        def cache_pair(p, h, b, i):
            for priority in (0, 1):
                r = priority * (win // 2) + i * _PIECE
                pltpu.make_async_copy(
                    caches[p].at[b, h, pl.ds(lo + r, _PIECE), :],
                    kv.at[p, b, pl.ds(r, _PIECE), :],
                    kvsem.at[p, b],
                ).start(priority=priority)

        def fetch_steps(p, h, b, with_weights):
            steps = [
                lambda i=i: cache_pair(p, h, b, i) for i in range(win // (2 * _PIECE))
            ]
            if with_weights:
                steps.insert(
                    len(steps) // 2, lambda: weight_pair(p, h + 1 if p == 3 else h, b)
                )
            return steps

        def spread(steps):
            per_chunk = [[] for _ in range(nchunk)]
            for i, step in enumerate(steps):
                per_chunk[i * nchunk // len(steps)].append(step)
            return per_chunk

        def wait_cache(p, b):
            pltpu.make_async_copy(kv.at[p, b], kv.at[p, b], kvsem.at[p, b]).wait()

        def wait_weights(m, h):
            pltpu.make_async_copy(wbuf.at[m, h], wbuf.at[m, h], wsem.at[m]).wait()

        def unit(br, h, h_next, next_q=True):
            pk, pv = 2 * br, 2 * br + 1
            mq, mo = (3, 0) if br == 0 else (1, 2)
            wait_weights(mq, h)
            q = lax.dot_general(xbuf[br], wbuf[mq, h], _NN, preferred_element_type=f32)
            q = jnp.where(row < nb, q[:, :dh], q[:, dh:]).astype(dt)

            def scores(b, carry):
                wait_cache(pk, b)
                fetch = spread(
                    [] if h_next is None else fetch_steps((pk + 2) % 4, h_next, b, True)
                )
                mine = (lax.broadcasted_iota(jnp.int32, (rows, _CHUNK), 0) & (nb - 1)) == b
                for c in range(nchunk):
                    for step in fetch[c]:
                        step()
                    sl = pl.ds(c * _CHUNK, _CHUNK)
                    s = lax.dot_general(q, kv[pk, b, sl, :], _NT, preferred_element_type=f32)
                    sbuf[:, sl] = jnp.where(mine, s, sbuf[:, sl])
                return carry

            lax.fori_loop(0, nb, scores, 0)
            s = sbuf[...] * (dh ** -0.5)
            e = jnp.exp(s - jnp.max(s, axis=1, keepdims=True))
            denom = jnp.sum(e, axis=1, keepdims=True)
            pbuf[...] = e

            def values(b, o):
                wait_cache(pv, b)
                fetch = spread(
                    [] if h_next is None else fetch_steps((pv + 2) % 4, h_next, b, next_q)
                )
                t = None
                for c in range(nchunk):
                    for step in fetch[c]:
                        step()
                    sl = pl.ds(c * _CHUNK, _CHUNK)
                    part = lax.dot_general(
                        pbuf[:, sl].astype(dt), kv[pv, b, sl, :], _NN,
                        preferred_element_type=f32,
                    )
                    t = part if t is None else t + part
                return jnp.where((row & (nb - 1)) == b, t, o)

            o = lax.fori_loop(0, nb, values, jnp.zeros((rows, dh), f32))
            o = (o / denom).astype(dt)
            wait_weights(mo, h)
            y0 = lax.dot_general(o, wbuf[mo, h, :, :dh], _NT, preferred_element_type=f32)
            y1 = lax.dot_general(o, wbuf[mo, h, :, dh:], _NT, preferred_element_type=f32)
            first = lax.broadcasted_iota(jnp.int32, (rows, d), 0) < nb
            acc[br] += jnp.where(first, y0, y1)

        def prologue(xraw):
            def first_wq(b, carry):
                weight_pair(3, 0, b)
                return carry

            lax.fori_loop(0, nb, first_wq, 0)
            copies = [
                pltpu.make_async_copy(x, xraw.at[i], xsem.at[i])
                for i, x in enumerate((xa, xb))
            ]
            for copy in copies:
                copy.start()
            for p in (0, 1):

                def first_windows(b, carry, p=p):
                    for step in fetch_steps(p, 0, b, True):
                        step()
                    return carry

                lax.fori_loop(0, nb, first_windows, 0)
            for i, copy in enumerate(copies):
                copy.wait()
                x = xraw[i].astype(f32)
                xbuf[i] = jnp.concatenate([x] * rep, axis=0).astype(dt)

        pl.run_scoped(prologue, pltpu.VMEM((2, nb, d), dt))
        acc[...] = jnp.zeros_like(acc)
        sbuf[...] = jnp.zeros_like(sbuf)

        def head(h, carry):
            unit(0, h, h)
            unit(1, h, h + 1)
            return carry

        lax.fori_loop(0, hkv - 1, head, 0)
        unit(0, hkv - 1, hkv - 1, next_q=False)
        unit(1, hkv - 1, None)
        total = acc[:, :nb] + acc[:, nb:]
        o_ref[...] = jnp.concatenate([total[0], total[1]], axis=1).astype(o_ref.dtype)

    out = pl.pallas_call(
        kernel,
        in_specs=[pl.BlockSpec(memory_space=pltpu.HBM)] * 10,
        out_specs=pl.BlockSpec(memory_space=pltpu.VMEM),
        out_shape=jax.ShapeDtypeStruct((nb, 2 * d), dt),
        scratch_shapes=[
            pltpu.VMEM((4, nb, win, dh), dt),
            pltpu.VMEM((4, hkv, d, hw), dt),
            pltpu.VMEM((2, rows, d), dt),
            pltpu.VMEM((rows, win), f32),
            pltpu.VMEM((rows, win), f32),
            pltpu.VMEM((2, rows, d), f32),
            pltpu.SemaphoreType.DMA((4, nb)),
            pltpu.SemaphoreType.DMA((4,)),
            pltpu.SemaphoreType.DMA((2,)),
        ],
        compiler_params=pltpu.CompilerParams(vmem_limit_bytes=64 * 1024 * 1024),
    )(
        A_x.reshape(nb, d), A_k_cache, A_v_cache, A_wq, A_wo.T,
        B_x.reshape(nb, d), B_k_cache, B_v_cache, B_wq, B_wo.T,
    )
    return out.reshape(nb, sq, 2 * d)
```

```python
import jax
import jax.numpy as jnp
from jax import lax
import jax.experimental.pallas as pl
import jax.experimental.pallas.tpu as pltpu

_HQ, _DH = 32, 128
_PAIRS = ((192, 160),) * 5 + ((128, 160),)
_LAST_COLS = 256
_NT = (((1,), (1,)), ((), ()))
_NN = (((1,), (0,)), ((), ()))


@jax.jit
def pallas_concat_heads__sliding_block_cached__sliding_block_cached__decode_kernel(
    A_x: jax.Array,
    A_k_cache: jax.Array,
    A_v_cache: jax.Array,
    A_wq: jax.Array,
    A_wo: jax.Array,
    B_x: jax.Array,
    B_k_cache: jax.Array,
    B_v_cache: jax.Array,
    B_wq: jax.Array,
    B_wo: jax.Array,
):
    nb, sq, d = A_x.shape
    _, hkv, sk, dh = A_k_cache.shape
    win = min(4096, max(256, sk // 4))
    rep = _HQ // hkv
    hw = rep * dh
    rows = rep * nb
    assert (sq, dh, rep, rows) == (1, _DH, 2, 8)
    assert win == sum(map(sum, _PAIRS)) and d % (16 * nb) == 0 and d > _LAST_COLS
    wrows = d // nb
    wsplit = wrows // 32 * 16
    f32, dt = jnp.float32, A_x.dtype

    def kernel(x0, k0, v0, wq0, wo0, x1, k1, v1, wq1, wo1, o_ref,
               kv, wbuf, xraw, xbuf, sbuf, pbuf, acc):
        caches = (k0, v0, k1, v1)
        weights = (wo0, wq1, wo1, wq0)

        def run(kvsem, wsem, xsem):
            row = lax.broadcasted_iota(jnp.int32, (rows, dh), 0)

            def weight_copy(m, h, r, n, sem):
                return pltpu.make_async_copy(
                    weights[m].at[pl.ds(r, n), pl.ds(pl.multiple_of(h * hw, hw), hw)],
                    wbuf.at[m, h, pl.ds(r, n), :],
                    sem,
                )

            def fetch_weights(m, h, b):
                for priority, (r, n) in enumerate(((0, wsplit), (wsplit, wrows - wsplit))):
                    r = pl.multiple_of(b * wrows + r, 16)
                    weight_copy(m, h, r, n, wsem.at[m]).start(priority=priority)

            def fetch(p, h, b, with_weights):
                offsets = [sum(n for _, n in _PAIRS), 0]
                for i, pair in enumerate(_PAIRS):
                    if with_weights and i == len(_PAIRS) // 2:
                        fetch_weights(p, h + 1 if p == 3 else h, b)
                    for priority, n in enumerate(pair):
                        r = offsets[priority]
                        offsets[priority] += n
                        pltpu.make_async_copy(
                            caches[p].at[b, h, pl.ds(sk - win + r, n), :],
                            kv.at[p, b, pl.ds(r, n), :],
                            kvsem.at[p, b],
                        ).start(priority=priority)

            def wait_cache(p, b):
                pltpu.make_async_copy(kv.at[p, b], kv.at[p, b], kvsem.at[p, b]).wait()

            def wait_weights(m, h):
                pltpu.make_async_copy(wbuf.at[m, h], wbuf.at[m, h], wsem.at[m]).wait()

            def attend(br, h, h_next, with_weights=True):
                pk, pv, mq = 2 * br, 2 * br + 1, 3 - 2 * br
                wait_weights(mq, h)
                q = lax.dot_general(xbuf[br], wbuf[mq, h], _NN, preferred_element_type=f32)
                q = jnp.where(row < nb, q[:, :dh], q[:, dh:]).astype(dt)

                def scores(b, carry):
                    wait_cache(pk, b)
                    if h_next is not None:
                        fetch((pk + 2) % 4, h_next, b, with_weights)
                    s = lax.dot_general(q, kv[pk, b], _NT, preferred_element_type=f32)
                    batch = lax.broadcasted_iota(jnp.int32, (rows, win), 0) & (nb - 1)
                    sbuf[...] = jnp.where(batch == b, s, sbuf[...])
                    return carry

                lax.fori_loop(0, nb, scores, 0)
                s = sbuf[...] * (dh ** -0.5)
                e = jnp.exp(s - jnp.max(s, axis=1, keepdims=True))
                denom = jnp.sum(e, axis=1, keepdims=True)
                pbuf[...] = e

                def values(b, o):
                    wait_cache(pv, b)
                    if h_next is not None:
                        fetch((pv + 2) % 4, h_next, b, with_weights)
                    t = lax.dot_general(
                        pbuf[...].astype(dt), kv[pv, b], _NN, preferred_element_type=f32
                    )
                    return jnp.where((row & (nb - 1)) == b, t, o)

                o = lax.fori_loop(0, nb, values, jnp.zeros((rows, dh), f32))
                return (o / denom).astype(dt)

            def project(o, m, h, r, n):
                y0, y1 = (
                    lax.dot_general(
                        o, wbuf[m, h, pl.ds(r, n), pl.ds(i * dh, dh)], _NT,
                        preferred_element_type=f32,
                    )
                    for i in range(rep)
                )
                return jnp.where(lax.broadcasted_iota(jnp.int32, (rows, n), 0) < nb, y0, y1)

            def unit(br, h, h_next, with_weights=True):
                o = attend(br, h, h_next, with_weights)
                wait_weights(2 * br, h)
                acc[br] += project(o, 2 * br, h, 0, d)

            def fold(y):
                return y[:nb] + y[nb:]

            def first_wq(b, carry):
                fetch_weights(3, 0, b)
                return carry

            lax.fori_loop(0, nb, first_wq, 0)
            x_copies = [
                pltpu.make_async_copy(x, xraw.at[i], xsem.at[i])
                for i, x in enumerate((x0, x1))
            ]
            for copy in x_copies:
                copy.start()
            for p in (0, 1):

                def first_windows(b, carry, p=p):
                    fetch(p, 0, b, True)
                    return carry

                lax.fori_loop(0, nb, first_windows, 0)
            for i, copy in enumerate(x_copies):
                copy.wait()
                xbuf[i] = jnp.concatenate([xraw[i].astype(f32)] * rep, axis=0).astype(dt)
            acc[...] = jnp.zeros_like(acc)
            sbuf[...] = jnp.zeros_like(sbuf)

            def head(h, carry):
                unit(0, h, h)
                unit(1, h, h + 1)
                return carry

            lax.fori_loop(0, hkv - 1, head, 0)

            h, cut = hkv - 1, _LAST_COLS
            unit(0, h, h, with_weights=False)
            early = weight_copy(2, h, cut, d - cut, wsem.at[2])
            final = weight_copy(2, h, 0, cut, wsem.at[0])
            early.start(priority=1)
            final.start(priority=1)
            o = attend(1, h, None)
            early.wait()
            y = fold(acc[1, :, cut:] + project(o, 2, h, cut, d - cut))
            o_ref[:, cut:] = jnp.concatenate([y, fold(acc[0])], axis=1).astype(dt)
            final.wait()
            o_ref[:, :cut] = fold(acc[1, :, :cut] + project(o, 2, h, 0, cut)).astype(dt)

        pl.run_scoped(
            run,
            pltpu.SemaphoreType.DMA((4, nb)),
            pltpu.SemaphoreType.DMA((4,)),
            pltpu.SemaphoreType.DMA((2,)),
        )

    out = pl.pallas_call(
        kernel,
        in_specs=[pl.BlockSpec(memory_space=pltpu.HBM)] * 10,
        out_specs=pl.BlockSpec(memory_space=pltpu.VMEM),
        out_shape=jax.ShapeDtypeStruct((nb, 2 * d), dt),
        scratch_shapes=[
            pltpu.VMEM((4, nb, win, dh), dt),
            pltpu.VMEM((4, hkv, d, hw), dt),
            pltpu.VMEM((2, nb, d), dt),
            pltpu.VMEM((2, rows, d), dt),
            pltpu.VMEM((rows, win), f32),
            pltpu.VMEM((rows, win), f32),
            pltpu.VMEM((2, rows, d), f32),
        ],
        compiler_params=pltpu.CompilerParams(vmem_limit_bytes=64 * 1024 * 1024),
    )(
        B_x.reshape(nb, d), B_k_cache, B_v_cache, B_wq, B_wo.T,
        A_x.reshape(nb, d), A_k_cache, A_v_cache, A_wq, A_wo.T,
    )
    return out.reshape(nb, sq, 2 * d)
```

```python
import jax
import jax.numpy as jnp
from jax import lax
import jax.experimental.pallas as pl
import jax.experimental.pallas.tpu as pltpu

_HQ, _DH = 32, 128
_PAIRS = (
    ((640, 192), (0, 160)),
    ((832, 192), (160, 160)),
    ((1024, 192), (320, 160)),
    ((1216, 192), (480, 160)),
    ((1408, 192), (1728, 160)),
    ((1600, 128), (1888, 160)),
)
_LAST_COLS = 256
_NT = (((1,), (1,)), ((), ()))
_NN = (((1,), (0,)), ((), ()))


@jax.jit
def pallas_concat_heads__sliding_block_cached__sliding_block_cached__decode_kernel(
    A_x: jax.Array,
    A_k_cache: jax.Array,
    A_v_cache: jax.Array,
    A_wq: jax.Array,
    A_wo: jax.Array,
    B_x: jax.Array,
    B_k_cache: jax.Array,
    B_v_cache: jax.Array,
    B_wq: jax.Array,
    B_wo: jax.Array,
):
    nb, sq, d = A_x.shape
    _, hkv, sk, dh = A_k_cache.shape
    win = min(4096, max(256, sk // 4))
    rep = _HQ // hkv
    hw = rep * dh
    rows = rep * nb
    assert (sq, dh, rep, rows) == (1, _DH, 2, 8)
    assert d % (16 * nb) == 0 and d > _LAST_COLS
    pieces = sorted(piece for pair in _PAIRS for piece in pair)
    assert [r for r, _ in pieces] + [win] == [0] + [r + n for r, n in pieces]
    wrows = d // nb
    wsplit = wrows // 24 * 16
    f32, dt = jnp.float32, A_x.dtype

    def kernel(x0, k0, v0, wq0, wo0, x1, k1, v1, wq1, wo1, o_ref,
               kv, wbuf, xraw, xbuf, sbuf, pbuf, acc):
        caches = (k0, v0, k1, v1)
        weights = (wo0, wq1, wo1, wq0)

        def run(kvsem, wsem, xsem):
            row = lax.broadcasted_iota(jnp.int32, (rows, dh), 0)

            def weight_copy(m, h, r, n, sem):
                return pltpu.make_async_copy(
                    weights[m].at[pl.ds(r, n), pl.ds(pl.multiple_of(h * hw, hw), hw)],
                    wbuf.at[m, h, pl.ds(r, n), :],
                    sem,
                )

            def fetch_weights(m, h, b, priorities):
                pair = ((0, wsplit), (wsplit, wrows - wsplit))
                for priority, (r, n) in zip(priorities, pair):
                    r = pl.multiple_of(b * wrows + r, 16)
                    weight_copy(m, h, r, n, wsem.at[m]).start(priority=priority)

            def fetch(p, h, b, with_weights, priorities=(0, 1)):
                for i, pair in enumerate(_PAIRS):
                    if with_weights and i == len(_PAIRS) // 2:
                        fetch_weights(p, h + 1 if p == 3 else h, b, priorities)
                    for priority, (r, n) in zip(priorities, pair):
                        pltpu.make_async_copy(
                            caches[p].at[b, h, pl.ds(sk - win + r, n), :],
                            kv.at[p, b, pl.ds(r, n), :],
                            kvsem.at[p, b],
                        ).start(priority=priority)

            def wait_cache(p, b):
                pltpu.make_async_copy(kv.at[p, b], kv.at[p, b], kvsem.at[p, b]).wait()

            def wait_weights(m, h):
                pltpu.make_async_copy(wbuf.at[m, h], wbuf.at[m, h], wsem.at[m]).wait()

            def attend(br, h, h_next, with_weights=True):
                pk, pv, mq = 2 * br, 2 * br + 1, 3 - 2 * br
                wait_weights(mq, h)
                q = lax.dot_general(xbuf[br], wbuf[mq, h], _NN, preferred_element_type=f32)
                q = jnp.where(row < nb, q[:, :dh], q[:, dh:]).astype(dt)

                def scores(b, carry):
                    wait_cache(pk, b)
                    if h_next is not None:
                        fetch((pk + 2) % 4, h_next, b, with_weights)
                    s = lax.dot_general(q, kv[pk, b], _NT, preferred_element_type=f32)
                    batch = lax.broadcasted_iota(jnp.int32, (rows, win), 0) & (nb - 1)
                    sbuf[...] = jnp.where(batch == b, s, sbuf[...])
                    return carry

                lax.fori_loop(0, nb, scores, 0)
                s = sbuf[...] * (dh ** -0.5)
                e = jnp.exp(s - jnp.max(s, axis=1, keepdims=True))
                denom = jnp.sum(e, axis=1, keepdims=True)
                pbuf[...] = e

                def values(b, o):
                    wait_cache(pv, b)
                    if h_next is not None:
                        fetch((pv + 2) % 4, h_next, b, with_weights)
                    t = lax.dot_general(
                        pbuf[...].astype(dt), kv[pv, b], _NN, preferred_element_type=f32
                    )
                    return jnp.where((row & (nb - 1)) == b, t, o)

                o = lax.fori_loop(0, nb, values, jnp.zeros((rows, dh), f32))
                return (o / denom).astype(dt)

            def project(o, m, h, r, n):
                y0, y1 = (
                    lax.dot_general(
                        o, wbuf[m, h, pl.ds(r, n), pl.ds(i * dh, dh)], _NT,
                        preferred_element_type=f32,
                    )
                    for i in range(rep)
                )
                return jnp.where(lax.broadcasted_iota(jnp.int32, (rows, n), 0) < nb, y0, y1)

            def unit(br, h, h_next, with_weights=True):
                o = attend(br, h, h_next, with_weights)
                wait_weights(2 * br, h)
                acc[br] += project(o, 2 * br, h, 0, d)

            def fold(y):
                return y[:nb] + y[nb:]

            def first_wq(b, carry):
                fetch_weights(3, 0, b, (1, 1))
                return carry

            lax.fori_loop(0, nb, first_wq, 0)
            x_copies = [
                pltpu.make_async_copy(x, xraw.at[i], xsem.at[i])
                for i, x in enumerate((x0, x1))
            ]
            for copy in x_copies:
                copy.start(priority=1)
            fetch(0, 0, 0, True, (1, 1))
            for p in (0, 1):

                def first_windows(b, carry, p=p):
                    fetch(p, 0, b, True)
                    return carry

                lax.fori_loop(1 - p, nb, first_windows, 0)
            for i, copy in enumerate(x_copies):
                copy.wait()
                xbuf[i] = jnp.concatenate([xraw[i].astype(f32)] * rep, axis=0).astype(dt)
            acc[...] = jnp.zeros_like(acc)
            sbuf[...] = jnp.zeros_like(sbuf)

            def head(h, carry):
                unit(0, h, h)
                unit(1, h, h + 1)
                return carry

            lax.fori_loop(0, hkv - 1, head, 0)

            h, cut = hkv - 1, _LAST_COLS
            unit(0, h, h, with_weights=False)
            early = weight_copy(2, h, cut, d - cut, wsem.at[2])
            final = weight_copy(2, h, 0, cut, wsem.at[0])
            early.start(priority=1)
            final.start(priority=1)
            o = attend(1, h, None)
            early.wait()
            y = fold(acc[1, :, cut:] + project(o, 2, h, cut, d - cut))
            o_ref[:, cut:] = jnp.concatenate([y, fold(acc[0])], axis=1).astype(dt)
            final.wait()
            o_ref[:, :cut] = fold(acc[1, :, :cut] + project(o, 2, h, 0, cut)).astype(dt)

        pl.run_scoped(
            run,
            pltpu.SemaphoreType.DMA((4, nb)),
            pltpu.SemaphoreType.DMA((4,)),
            pltpu.SemaphoreType.DMA((2,)),
        )

    out = pl.pallas_call(
        kernel,
        in_specs=[pl.BlockSpec(memory_space=pltpu.HBM)] * 10,
        out_specs=pl.BlockSpec(memory_space=pltpu.VMEM),
        out_shape=jax.ShapeDtypeStruct((nb, 2 * d), dt),
        scratch_shapes=[
            pltpu.VMEM((4, nb, win, dh), dt),
            pltpu.VMEM((4, hkv, d, hw), dt),
            pltpu.VMEM((2, nb, d), dt),
            pltpu.VMEM((2, rows, d), dt),
            pltpu.VMEM((rows, win), f32),
            pltpu.VMEM((rows, win), f32),
            pltpu.VMEM((2, rows, d), f32),
        ],
        compiler_params=pltpu.CompilerParams(vmem_limit_bytes=64 * 1024 * 1024),
    )(
        B_x.reshape(nb, d), B_k_cache, B_v_cache, B_wq, B_wo.T,
        A_x.reshape(nb, d), A_k_cache, A_v_cache, A_wq, A_wo.T,
    )
    return out.reshape(nb, sq, 2 * d)
```
